```python
import jax
import jax.numpy as jnp

def _softmax(x, axis=-1):
    return jax.nn.softmax(x, axis=axis)
def _gelu(x):
    return jax.nn.gelu(x, approximate=True)
def _silu(x):
    return jax.nn.silu(x)
def _sigmoid(x):
    return jax.nn.sigmoid(x)
def _layernorm(x, axis=-1, eps=1e-5):
    m = jnp.mean(x, axis=axis, keepdims=True)
    v = jnp.var(x, axis=axis, keepdims=True)
    return (x - m) / jnp.sqrt(v + eps)
def _scatter_add(tgt, idx, src, axis=0):
    return tgt.at[idx].add(src)
def _segment_sum(src, seg, n):
    return jax.ops.segment_sum(src, seg, n)
class _Rng:
    def __init__(self, key):
        self._k = key
    def _next(self):
        self._k, sub = jax.random.split(self._k)
        return sub
    def normal(self, shape):
        return jax.random.normal(self._next(), shape, dtype=jnp.bfloat16)
    def randint(self, lo, hi, shape):
        return jax.random.randint(self._next(), shape, lo, hi, dtype=jnp.int32)
    def uniform(self, shape, lo=0.0, hi=1.0):
        return jax.random.uniform(self._next(), shape, jnp.bfloat16, lo, hi)
    def permutation(self, n):
        return jax.random.permutation(self._next(), n)


kernel_name = 'standalone__fused_io_aware_attn__prompt'

def setup_inputs():
    _rng = _Rng(jax.random.key(int.from_bytes(__import__("os").urandom(4), "little")))
    _w = (lambda a: (lambda t: t.astype(jnp.bfloat16) if jnp.issubdtype(t.dtype, jnp.floating) else t)(jnp.asarray(a)))
    B, H, S = 2, 32, 2048
    Dh = max(1, 1024 // 32)
    return {
        "q": _w((lambda *s: _rng.normal(s) * 0.05)(B, H, S, Dh)),
        "k": _w((lambda *s: _rng.normal(s) * 0.05)(B, H, S, Dh)),
        "v": _w((lambda *s: _rng.normal(s) * 0.05)(B, H, S, Dh)),
    }

def reference(q, k, v):
    scale = q.shape[-1] ** -0.5
    s = jnp.einsum('bhqd,bhkd->bhqk', q, k) * scale
    p = _softmax(s, axis=-1)
    return jnp.einsum('bhqk,bhkd->bhqd', p, v)
```

```python
import math

import jax
import jax.numpy as jnp
from jax import lax
import jax.experimental.pallas as pl
import jax.experimental.pallas.tpu as pltpu

f32, bf16, u32 = jnp.float32, jnp.bfloat16, jnp.uint32

_BK = 256
_HB = 2
_SAFE_LOG2 = 30.0


def _prep_chunk(q_ref, k_ref, k2_ref, q2_ref, c0, cw, nrm):
    d = q_ref.shape[0]
    cs = slice(c0, c0 + cw)
    qc = q_ref[:, cs].astype(f32) * (d ** -0.5 * math.log2(math.e))
    hi = qc.astype(bf16)
    lo = (qc - hi.astype(f32)).astype(bf16)
    q2_ref[0:d // 2, cs] = pltpu.bitcast(hi, u32)
    q2_ref[d // 2:d, cs] = pltpu.bitcast(lo, u32)
    kt = k_ref[:, cs]
    k2_ref[c0 // 2:(c0 + cw) // 2, :] = pltpu.bitcast(jnp.concatenate([kt, kt], axis=0).T, u32)

    def nmax(x, m):
        n = jnp.sum(x * x, axis=0, keepdims=True)
        for i in range(cw // 128):
            t = n[:, i * 128:(i + 1) * 128]
            m = t if m is None else jnp.maximum(m, t)
        return m

    return nmax(qc, nrm[0]), nmax(kt.astype(f32), nrm[1])


def _fast(k2_ref, q2_ref, nrm_ref, v_ref, o_ref, nxt):
    qn_ref, kn_ref, k2n_ref, q2n_ref, nrmn_ref = nxt
    d, s = v_ref.shape
    nrm = (None, None)
    vm = None
    qt = pltpu.bitcast(q2_ref[...], bf16)
    acc = jnp.zeros((d, s), f32)
    l = jnp.zeros((8, s), f32)
    for kj in range(s // _BK):
        kb = pltpu.bitcast(k2_ref[kj * _BK // 2:(kj + 1) * _BK // 2, :], bf16)
        p = jnp.exp2(jnp.dot(kb, qt, preferred_element_type=f32))
        l = l + p.reshape(_BK // 8, 8, s).sum(axis=0)
        vb = v_ref[:, kj * _BK:(kj + 1) * _BK]
        acc = acc + jnp.dot(vb, p.astype(bf16), preferred_element_type=f32)
        nrm = _prep_chunk(qn_ref, kn_ref, k2n_ref, q2n_ref, kj * _BK, _BK, nrm)
        va = jnp.abs(vb.astype(f32)).reshape(d // 8, 8, _BK).max(axis=0)
        for i in range(_BK // 128):
            t = va[:, i * 128:(i + 1) * 128]
            vm = t if vm is None else jnp.maximum(vm, t)
    lt = jnp.sum(l, axis=0, keepdims=True)
    o_ref[...] = (acc * (1.0 / lt)).astype(o_ref.dtype)
    nr = nrm_ref[0:2, :]
    bound2 = jnp.max(nr[0:1, :]) * jnp.max(nr[1:2, :])
    vmax = jnp.max(vm)
    nrmn_ref[0:1, :] = nrm[0]
    nrmn_ref[1:2, :] = nrm[1]
    return (bound2 <= _SAFE_LOG2 ** 2) & (vmax <= 2.0 ** 60) & (vmax >= 2.0 ** -60)


def _slow(k2_ref, q2_ref, v_ref, o_ref):
    d, s = v_ref.shape
    sq = sk = 256

    def qloop(qi, carry):
        q0 = pl.multiple_of(qi * sq, sq)
        qt = pltpu.bitcast(q2_ref[:, pl.ds(q0, sq)], bf16)

        def kloop(kj, mla):
            m, l, acc = mla
            kb = pltpu.bitcast(k2_ref[pl.ds(pl.multiple_of(kj * (sk // 2), sk // 2), sk // 2), :], bf16)
            sc = jnp.dot(kb, qt, preferred_element_type=f32)
            mn = jnp.maximum(m, jnp.max(sc, axis=0, keepdims=True))
            a = jnp.exp2(m - mn)
            p = jnp.exp2(sc - mn)
            l = a * l + jnp.sum(p, axis=0, keepdims=True)
            vb = v_ref[:, pl.ds(pl.multiple_of(kj * sk, sk), sk)]
            acc = a * acc + jnp.dot(vb, p.astype(bf16), preferred_element_type=f32)
            return mn, l, acc

        init = (jnp.full((1, sq), -jnp.inf, f32), jnp.zeros((1, sq), f32), jnp.zeros((d, sq), f32))
        _, l, acc = lax.fori_loop(0, s // sk, kloop, init)
        o_ref[:, pl.ds(q0, sq)] = (acc / l).astype(o_ref.dtype)
        return carry

    lax.fori_loop(0, s // sq, qloop, 0)


def _kernel(q_hbm, k_hbm, *refs):
    qn, kn = refs[:_HB], refs[_HB:2 * _HB]
    v_ref, o_ref, k2a, q2a, nra, k2b, q2b, nrb, qs, ks, sem = refs[2 * _HB:]
    step = pl.program_id(0)

    def first(_, carry):
        cq = pltpu.make_async_copy(q_hbm.at[0], qs, sem.at[0])
        ck = pltpu.make_async_copy(k_hbm.at[0], ks, sem.at[1])
        cq.start()
        ck.start()
        cq.wait()
        ck.wait()
        nrm = (None, None)
        for c in range(qs.shape[1] // _BK):
            nrm = _prep_chunk(qs, ks, k2a, q2a, c * _BK, _BK, nrm)
        nra[0:1, :] = nrm[0]
        nra[1:2, :] = nrm[1]
        return carry

    lax.fori_loop(0, jnp.where(step == 0, 1, 0), first, 0)

    slots = [(k2a, q2a, nra), (k2b, q2b, nrb)]
    for h in range(_HB):
        k2, q2, nr = slots[h % 2]
        ok = _fast(k2, q2, nr, v_ref.at[h], o_ref.at[h], (qn[h], kn[h]) + slots[1 - h % 2])

        @pl.when(jnp.logical_not(ok))
        def _():
            _slow(k2, q2, v_ref.at[h], o_ref.at[h])


@jax.jit
def pallas_standalone__fused_io_aware_attn__prompt_kernel(
    q: jax.Array,
    k: jax.Array,
    v: jax.Array,
):
    b, h, s, d = q.shape
    n = b * h
    qt, kt, vt = (jnp.swapaxes(x, 2, 3).reshape(n, d, s) for x in (q, k, v))
    cur = pl.BlockSpec((_HB, d, s), lambda i: (i, 0, 0))
    nxt = [pl.BlockSpec((None, d, s), lambda i, j=j: (jnp.minimum(_HB * i + j + 1, n - 1), 0, 0))
           for j in range(_HB)]
    hbm = pl.BlockSpec(memory_space=pl.ANY)
    slot = [pltpu.VMEM((s // 2, 2 * d), u32), pltpu.VMEM((d, s), u32), pltpu.VMEM((8, 128), f32)]
    ot = pl.pallas_call(
        _kernel,
        out_shape=jax.ShapeDtypeStruct((n, d, s), q.dtype),
        grid=(n // _HB,),
        in_specs=[hbm, hbm] + nxt + nxt + [cur],
        out_specs=cur,
        scratch_shapes=slot + slot + [pltpu.VMEM((d, s), bf16)] * 2 + [pltpu.SemaphoreType.DMA((2,))],
        compiler_params=pltpu.CompilerParams(dimension_semantics=("arbitrary",)),
    )(qt, kt, *([qt] * _HB), *([kt] * _HB), vt)
    return jnp.swapaxes(ot.reshape(b, h, d, s), 2, 3)
```
